```python
import os as _os
_os.environ.setdefault("JAX_PLATFORMS", "cpu")
import jax
import jax.numpy as jnp

def _softmax(x, axis=-1):
    return jax.nn.softmax(x, axis=axis)
def _gelu(x):
    return jax.nn.gelu(x, approximate=True)
def _silu(x):
    return jax.nn.silu(x)
def _sigmoid(x):
    return jax.nn.sigmoid(x)
def _layernorm(x, axis=-1, eps=1e-5):
    m = jnp.mean(x, axis=axis, keepdims=True)
    v = jnp.var(x, axis=axis, keepdims=True)
    return (x - m) / jnp.sqrt(v + eps)
def _scatter_add(tgt, idx, src, axis=0):
    return tgt.at[idx].add(src)
def _segment_sum(src, seg, n):
    return jax.ops.segment_sum(src, seg, n)
class _Rng:
    def __init__(self, key):
        self._k = key
    def _next(self):
        self._k, sub = jax.random.split(self._k)
        return sub
    def normal(self, shape):
        return jax.random.normal(self._next(), shape, dtype=jnp.bfloat16)
    def randint(self, lo, hi, shape):
        return jax.random.randint(self._next(), shape, lo, hi, dtype=jnp.int32)
    def uniform(self, shape, lo=0.0, hi=1.0):
        return jax.random.uniform(self._next(), shape, jnp.bfloat16, lo, hi)
    def permutation(self, n):
        return jax.random.permutation(self._next(), n)


kernel_name = 'sequential_preLN__ssm_conv_h3__mixer_channel_mlp__prompt'

def setup_inputs():
    _rng = _Rng(jax.random.key(int.from_bytes(__import__("os").urandom(4), "little")))
    _w = (lambda a: (lambda t: t.astype(jnp.bfloat16) if jnp.issubdtype(t.dtype, jnp.floating) else t)(jnp.asarray(a)))
    def _A_setup():
        B, S, D = 1, 2048, 448
        ks = 4
        return {
            "q": _w((lambda *s: _rng.normal(s) * 0.05)(B, S, D)),
            "k": _w((lambda *s: _rng.normal(s) * 0.05)(B, S, D)),
            "v": _w((lambda *s: _rng.normal(s) * 0.05)(B, S, D)),
            "shift_k": _w((lambda *s: _rng.normal(s) * 0.05)(D, ks) * 0.5),
            "ssm_k": _w((lambda *s: _rng.normal(s) * 0.05)(D, S) * (1.0 / S ** 0.5)),
            "ssm_D": _w((lambda *s: _rng.normal(s) * 0.05)(D)),
        }
    _A_in = _A_setup()

    def _B_setup():
        B, S, D, F = 1, 2048, 448, 1792
        return {
            "x": _w((lambda *s: _rng.normal(s) * 0.05)(B, S, D)),
            "w1": _w((lambda *s: _rng.normal(s) * 0.2)(D, F) * (D ** -0.5)),
            "b1": _w((lambda *s: _rng.normal(s) * 0.2)(F)),
            "w2": _w((lambda *s: _rng.normal(s) * 0.2)(F, D) * (F ** -0.5)),
            "b2": _w((lambda *s: _rng.normal(s) * 0.05)(D)),
        }
    _B_in = _B_setup()

    return {
        "A_q": _A_in["q"],
        "A_k": _A_in["k"],
        "A_v": _A_in["v"],
        "A_shift_k": _A_in["shift_k"],
        "A_ssm_k": _A_in["ssm_k"],
        "A_ssm_D": _A_in["ssm_D"],
        "B_x": _B_in["x"],
        "B_w1": _B_in["w1"],
        "B_b1": _B_in["b1"],
        "B_w2": _B_in["w2"],
        "B_b2": _B_in["b2"],
    }

def reference(A_q, A_k, A_v, A_shift_k, A_ssm_k, A_ssm_D, B_x, B_w1, B_b1, B_w2, B_b2):
    def _A_ref(q, k, v, shift_k, ssm_k, ssm_D):
        B, S, D = q.shape
        ks = shift_k.shape[-1]
        k_pad = jnp.pad(k, ((0, 0), (ks - 1, 0), (0, 0)))
        k_shift = jnp.zeros_like(k)
        for t in range(ks):
            k_shift = k_shift + k_pad[:, t:t + S, :] * shift_k[:, ks - 1 - t][None, None, :]
        kv = k_shift * v
        L = 2 * S
        kv_pad = jnp.pad(kv, ((0, 0), (0, S), (0, 0)))
        kf_pad = jnp.pad(ssm_k, ((0, 0), (0, S)))
        kv_f = (lambda x, axes=(-2,-1): jnp.fft.rfft2(x.astype(jnp.float32), axes=axes))(kv_pad[:, None, :, :], axes=(1, 2))
        kf_f = (lambda x, axes=(-2,-1): jnp.fft.rfft2(x.astype(jnp.float32), axes=axes))(kf_pad[:, None, :], axes=(1, 2))
        kf_f = (lambda x, *d: x.transpose(*d))(kf_f, 1, 2, 0)
        y_f = kv_f * kf_f[None, :, :, :]
        y = (lambda x, s, axes=(-2,-1): jnp.fft.irfft2(x, s=s, axes=axes).astype(jnp.bfloat16))(y_f, (1, L), axes=(1, 2))[:, 0, :S, :]
        y = y + kv * ssm_D[None, None, :]
        return q * y

    def _B_ref(x, w1, b1, w2, b2):
        y = _layernorm(x, axis=-1)
        h = _gelu(jnp.einsum("bsd,df->bsf", y, w1) + b1)
        return jnp.einsum("bsf,fd->bsd", h, w2) + b2

    x = A_q
    h = x + _A_ref(_layernorm(x, axis=-1), A_k, A_v, A_shift_k, A_ssm_k, A_ssm_D)
    h2 = h + _B_ref(_layernorm(h, axis=-1), B_w1, B_b1, B_w2, B_b2)
    return h2
```

```python
import functools, contextlib
import numpy as np
import jax
import jax.numpy as jnp
from jax.experimental import pallas as pl
from jax.experimental.pallas import tpu as pltpu

S, D, F = 2048, 448, 1792
C = 128
NC = S // C
DP = 512
C0 = float(np.sqrt(2 / np.pi)); C1 = C0 * 0.044715
f32, bf16 = jnp.float32, jnp.bfloat16

def _dft_np():
    b = np.arange(C)[:, None].astype(np.float64); m = np.arange(C)[None, :].astype(np.float64)
    th = 2 * np.pi * (m + 0.25) / C * b
    Ff = np.concatenate([np.cos(th), np.sin(th)], 1)
    return Ff.astype(np.float32), (Ff.T / C).astype(np.float32)
_FF, _GI = _dft_np()

def make(blocks=(4, 4, 2, 2, 2, 2), gauss=True, nobar=2, AG=8, mix=True, gate=False):
    nb = len(blocks)
    starts = [int(v) for v in np.cumsum((0,) + tuple(blocks))[:-1]]
    TM = max(blocks) * C
    NV = 3 if gauss else 2

    def kern(q_h, k_h, v_h, sk_h, w1_h, w2_h, shk_ref, sd_ref, b1_ref, b2_ref, ff_ref, gi_ref, one_ref,
             o_h,
             q_v, k_v, v_v, sk_v, w1_v, w1T, w2P, w2T, shB, Xs, Ks, Kraw, Ys, uT, hT, hn, dB, b2B, o_v, sems):
        def cp(src, dst, i):
            return pltpu.make_async_copy(src, dst, sems.at[i])
        def in_copies(s):
            t0, T = starts[s] * C, blocks[s] * C
            return [cp(k_h.at[:, pl.ds(t0, T)], k_v.at[:, pl.ds(t0, T)], 4 * s),
                    cp(v_h.at[:, pl.ds(t0, T)], v_v.at[:, pl.ds(t0, T)], 4 * s + 1),
                    cp(sk_h.at[:, pl.ds(t0, T)], sk_v.at[:, pl.ds(t0, T)], 4 * s + 2),
                    cp(q_h.at[:, pl.ds(t0, T)], q_v.at[:, pl.ds(t0, T)], 4 * s + 3)]
        w1c = cp(w1_h, w1_v, 4 * nb); w2c = cp(w2_h, w2T, 4 * nb + 1)
        def out_copy(s):
            t0, T = starts[s] * C, blocks[s] * C
            return cp(o_v.at[:, pl.ds(t0, T)], o_h.at[:, pl.ds(t0, T)], 4 * nb + 2 + s)
        for c in in_copies(0): c.start()
        for j in range(4):
            shB[j] = jnp.broadcast_to(shk_ref[j:j + 1, :].astype(f32), (C, D)).T
        dB[...] = jnp.broadcast_to(sd_ref[...].astype(f32).reshape(1, D), (C, D)).T
        b2B[...] = jnp.broadcast_to(b2_ref[...].astype(f32).reshape(1, D), (C, D)).T
        rid = jax.lax.broadcasted_iota(jnp.int32, (DP - D, TM), 0)
        hn[0, D:DP, :] = jnp.where(rid == 0, 1.0, 0.0).astype(bf16)
        hn[1, D:DP, :] = jnp.where(rid == 0, 1.0, 0.0).astype(bf16)

        def prep_w1():
            w1c.wait()
            rid = jax.lax.broadcasted_iota(jnp.int32, (DP - D, 256), 0)
            for c in range(F // 256):
                sl = slice(c * 256, (c + 1) * 256)
                pad = jnp.where(rid == 0, b1_ref[...].astype(f32).reshape(1, F)[:, sl], 0.0).astype(bf16)
                blk = jnp.concatenate([w1_v[:, sl], pad], axis=0)
                w1T[c * 128:(c + 1) * 128, :] = pltpu.bitcast(blk.T, jnp.int32)
        def prep_w2():
            w2c.wait()

        RG = D // 7; FC = F // 7
        def conv_group(s, g):
            a0, n = starts[s], blocks[s]; t0 = a0 * C
            r = slice(g * RG, (g + 1) * RG)
            lane = jax.lax.broadcasted_iota(jnp.int32, (RG, C), 1)
            kvs = []
            sh_ = [shB[j, r, :] for j in range(4)]
            prev = None
            if a0 > 0:
                kp = k_v[r, t0 - C:t0].astype(f32)
                prev = [pltpu.roll(kp, j, 1) for j in range(1, 4)]
            for i in range(n):
                cs_ = slice(t0 + i * C, t0 + (i + 1) * C)
                kc_ = k_v[r, cs_].astype(f32)
                rolled = [pltpu.roll(kc_, j, 1) for j in range(1, 4)]
                ks = kc_ * sh_[0]
                for j in range(1, 4):
                    ks = ks + jnp.where(lane >= j, rolled[j - 1], 0.0 if prev is None else prev[j - 1]) * sh_[j]
                prev = rolled
                kvs.append((ks * v_v[r, cs_].astype(f32)).astype(bf16))
                yield
            lhs = jnp.concatenate(kvs + [sk_v[r, (a0 + i) * C:(a0 + i + 1) * C] for i in range(n)], axis=0)
            z = jnp.dot(lhs, ff_ref[...], preferred_element_type=f32)
            def put(ref, a, zr, zi, isx):
                if not gauss: vs = [zr, zi]
                elif isx: vs = [zr + zi, zr, zi]
                else: vs = [zr, zi - zr, zr + zi]
                for v in range(NV): ref[a, r, v * C:(v + 1) * C] = vs[v]
            for i in range(n):
                zz = z[i * RG:(i + 1) * RG]; put(Xs, a0 + i, zz[:, :C], zz[:, C:], True)
                yield
            zp = Kraw[r, :] if a0 > 0 else None
            for i in range(n):
                z0 = z[(n + i) * RG:(n + i + 1) * RG]
                if zp is None: put(Ks, a0 + i, z0[:, :C], z0[:, C:], False)
                else: put(Ks, a0 + i, z0[:, :C] + zp[:, C:], z0[:, C:] - zp[:, :C], False)
                zp = z0
                yield
            Kraw[r, :] = zp
            d_ = dB[r, :]
            for i in range(n):
                uT[s % 2, r, i * C:(i + 1) * C] = kvs[i].astype(f32) * d_

        def conv_acc(s, g):
            a0, n = starts[s], blocks[s]
            r = slice(g * RG, (g + 1) * RG)
            yy = []
            for q in range(RG // AG):
                rr = slice(g * RG + q * AG, g * RG + (q + 1) * AG)
                acc = [[None] * NV for _ in range(n)]
                kc = {}
                def ld(ref, a): return [ref[a, rr, v * C:(v + 1) * C] for v in range(NV)]
                def add(x, y): return y if x is None else x + y
                for ap in range(a0 + n - 1, -1, -1):
                    x = ld(Xs, ap)
                    for i in range(n):
                        j = a0 + i - ap
                        if j < 0: continue
                        if j not in kc: kc[j] = ld(Ks, j)
                        kk = kc[j]
                        if gauss:
                            for v in range(3): acc[i][v] = add(acc[i][v], kk[v] * x[v])
                        else:
                            acc[i][0] = add(acc[i][0], kk[0] * x[0] - kk[1] * x[1])
                            acc[i][1] = add(acc[i][1], kk[0] * x[1] + kk[1] * x[0])
                ys = []
                for i in range(n):
                    if gauss: yr, yi = acc[i][0] - acc[i][2], acc[i][0] + acc[i][1]
                    else: yr, yi = acc[i]
                    ys.append(jnp.concatenate([yr, yi], axis=1))
                yy.append(ys)
                yield
            ys = [jnp.concatenate([yq[i] for yq in yy], axis=0) for i in range(n)]
            Ys[(s * 7 + g) % 2, 0:n * RG, :] = jnp.concatenate(ys, axis=0).astype(bf16)

        def conv_inv(s, g):
            n = blocks[s]
            r = slice(g * RG, (g + 1) * RG)
            y = jnp.dot(Ys[(s * 7 + g) % 2, 0:n * RG, :], gi_ref[...], preferred_element_type=f32)
            for i in range(n):
                uT[s % 2, r, i * C:(i + 1) * C] += y[i * RG:(i + 1) * RG]
            yield

        def lnT(h):
            m = jnp.sum(h, 0, keepdims=True) * (1.0 / D); c = h - m
            v = jnp.sum(c * c, 0, keepdims=True) * (1.0 / D)
            return c * jax.lax.rsqrt(v + 1e-5)

        def ln_chunk(s, i):
            t0 = (starts[s] + i) * C
            cs = slice(i * C, (i + 1) * C)
            x = q_v[:, t0:t0 + C].astype(f32)
            xn = lnT(x)
            yield
            h = x + xn * uT[s % 2, :, cs]
            hT[s % 2, :, cs] = h + b2B[...]
            yield
            hn[s % 2, 0:D, cs] = lnT(h).astype(bf16)
            yield

        def gelu(z):
            u = z * (C0 + C1 * (z * z)); hz = 0.5 * z
            return (hz * jnp.tanh(u) + hz).astype(bf16)

        for rd in range(nb + 2):
            sc, sl_, sm = rd, rd - 1, rd - 2
            if rd == 0:
                for c in in_copies(0)[:3]: c.wait()
                for _ in conv_group(0, 0): pass
            if 0 <= sl_ < nb: in_copies(sl_)[3].wait()
            if rd + 1 < nb:
                for cc in in_copies(rd + 1): cc.start()
            if rd == 0: w1c.start()
            if rd == 1: w2c.start()
            if rd == 2:
                w2c.wait()
                w2P[...] = pltpu.bitcast(w2T[...], jnp.int32)
            if sm >= 0:
                T = blocks[sm] * C; t0 = starts[sm] * C
                z = None
            for c in range(7):
                if c == 5 and sc + 1 < nb:
                    for cc in in_copies(sc + 1)[:3]: cc.wait()
                if True:
                    gens = []; cnt = 0
                    t = sc * 7 + c
                    if 0 <= t - 1 < nb * 7: gens.append(conv_inv(*divmod(t - 1, 7))); cnt += 1
                    if t + 1 < nb * 7: gens.append(conv_group(*divmod(t + 1, 7))); cnt += 3 * blocks[(t + 1) // 7]
                    if 0 <= sl_ < nb:
                        for i in range(blocks[sl_]):
                            if 1 + i * 6 // blocks[sl_] == c: gens.append(ln_chunk(sl_, i)); cnt += 3
                    if t < nb * 7: gens.append(conv_acc(sc, c)); cnt += RG // AG
                    def rr_():
                        gl = list(gens)
                        if mix:
                            while gl:
                                for g_ in list(gl):
                                    try: next(g_); yield
                                    except StopIteration: gl.remove(g_)
                        else:
                            for g_ in gl: yield from g_
                    it = rr_()
                    def fill(k, val):
                        nr = val.shape[0]
                        for j in range(k):
                            r0 = (j * nr // k) // 16 * 16
                            if gate:
                                Xs[one_ref[0], 0:8, 0:C] = val[r0:r0 + 8, 0:C]
                                gsl = pl.ds(pl.multiple_of(one_ref[1], C), C)
                                vb = val[r0:r0 + 16, 0:C].astype(bf16)
                            next(it, None)
                    if sm >= 0:
                        n = blocks[sm]
                        nu = (n if c < 6 else 0) + 2 * ((n + 1) // 2); per = -(-cnt // nu)
                        d1 = lambda c, i: jnp.dot(pltpu.bitcast(w1T[c * FC // 2:(c + 1) * FC // 2, :], bf16), hn[sm % 2, :, i * C:(i + 1) * C], preferred_element_type=f32)
                        if c == 0: z = [d1(0, i) for i in range(n)]
                        gs = []
                        for i in range(n):
                            zo = z[i]
                            if c < 6:
                                z[i] = d1(c + 1, i)
                                fill(per, z[i])
                            gs.append(gelu(zo))
                            if i % 2 == 1 or i == n - 1:
                                w = len(gs) * C; cs = slice((i + 1) * C - w, (i + 1) * C)
                                p = jnp.dot(pltpu.bitcast(w2P[:, c * FC:(c + 1) * FC], bf16), jnp.concatenate(gs, axis=1), preferred_element_type=f32)
                                gs = []
                                fill(2 * per, p)
                                if c < 6: hT[sm % 2, :, cs] += p
                                else: o_v[:, t0 + cs.start:t0 + cs.stop] = (hT[sm % 2, :, cs] + p).astype(bf16)
                        if c == 6: out_copy(sm).start()
                    for _ in it: pass
                    if rd == 1 and c == 3: prep_w1()
        for s in range(nb): out_copy(s).wait()

    anyspec = pl.BlockSpec(memory_space=pltpu.MemorySpace.HBM)
    vm = pl.BlockSpec(memory_space=pltpu.VMEM)
    call = pl.pallas_call(
        kern,
        in_specs=[anyspec] * 6 + [vm] * 6 + [pl.BlockSpec(memory_space=pltpu.SMEM)],
        out_specs=anyspec,
        out_shape=jax.ShapeDtypeStruct((D, S), bf16),
        scratch_shapes=[
            pltpu.VMEM((D, S + C), bf16), pltpu.VMEM((D, S + C), bf16), pltpu.VMEM((D, S), bf16), pltpu.VMEM((D, S), bf16),
            pltpu.VMEM((D, F), bf16), pltpu.VMEM((F // 2, DP), jnp.int32), pltpu.VMEM((D // 2, F), jnp.int32), pltpu.VMEM((D, F), bf16),
            pltpu.VMEM((4, D, C), f32),
            pltpu.VMEM((NC + 1, D, NV * C), f32), pltpu.VMEM((NC, D, NV * C), f32),
            pltpu.VMEM((D, 2 * C), f32), pltpu.VMEM((2, max(blocks) * 64, 2 * C), bf16), pltpu.VMEM((2, D, TM), f32), pltpu.VMEM((2, D, TM), f32), pltpu.VMEM((2, DP, TM), bf16),
            pltpu.VMEM((D, C), f32), pltpu.VMEM((D, C), f32),
            pltpu.VMEM((D, S), bf16),
            pltpu.SemaphoreType.DMA((5 * nb + 2,)),
        ],
        compiler_params=pltpu.CompilerParams(vmem_limit_bytes=110 * 2**20),
    )
    def fn(A_q, A_k, A_v, A_shift_k, A_ssm_k, A_ssm_D, B_x, B_w1, B_b1, B_w2, B_b2):
        o = call(A_q.reshape(S, D).T, A_k.reshape(S, D).T, A_v.reshape(S, D).T, A_ssm_k, B_w1, B_w2.T,
                 A_shift_k.T, A_ssm_D, B_b1, B_b2,
                 jnp.asarray(_FF, bf16), jnp.asarray(_GI, bf16), jnp.asarray(np.array([NC, S], np.int32)))
        return o.T.reshape(1, S, D)
    return fn


@jax.jit
def pallas_sequential_preLN__ssm_conv_h3__mixer_channel_mlp__prompt_kernel(A_q, A_k, A_v, A_shift_k, A_ssm_k, A_ssm_D, B_x, B_w1, B_b1, B_w2, B_b2):
    return make()(A_q, A_k, A_v, A_shift_k, A_ssm_k, A_ssm_D, B_x, B_w1, B_b1, B_w2, B_b2)
```
